```python
import jax
import jax.numpy as jnp

def _softmax(x, axis=-1):
    return jax.nn.softmax(x, axis=axis)
def _gelu(x):
    return jax.nn.gelu(x, approximate=True)
def _silu(x):
    return jax.nn.silu(x)
def _sigmoid(x):
    return jax.nn.sigmoid(x)
def _layernorm(x, axis=-1, eps=1e-5):
    m = jnp.mean(x, axis=axis, keepdims=True)
    v = jnp.var(x, axis=axis, keepdims=True)
    return (x - m) / jnp.sqrt(v + eps)
def _scatter_add(tgt, idx, src, axis=0):
    return tgt.at[idx].add(src)
def _segment_sum(src, seg, n):
    return jax.ops.segment_sum(src, seg, n)
class _Rng:
    def __init__(self, key):
        self._k = key
    def _next(self):
        self._k, sub = jax.random.split(self._k)
        return sub
    def normal(self, shape):
        return jax.random.normal(self._next(), shape, dtype=jnp.bfloat16)
    def randint(self, lo, hi, shape):
        return jax.random.randint(self._next(), shape, lo, hi, dtype=jnp.int32)
    def uniform(self, shape, lo=0.0, hi=1.0):
        return jax.random.uniform(self._next(), shape, jnp.bfloat16, lo, hi)
    def permutation(self, n):
        return jax.random.permutation(self._next(), n)


kernel_name = 'gated_mix__sliding_block_cached__glu_gated_swiglu__decode'

def setup_inputs():
    _rng = _Rng(jax.random.key(int.from_bytes(__import__("os").urandom(4), "little")))
    _w = (lambda a: (lambda t: t.astype(jnp.bfloat16) if jnp.issubdtype(t.dtype, jnp.floating) else t)(jnp.asarray(a)))
    def _A_setup():
        B, Sq, D = 1, 1, 640
        Hq, Hkv, Sk, Dh = 32, 32, 32768, 192
        assert Hq % Hkv == 0, (Hq, Hkv)
        return {
            "x": _w((lambda *s: _rng.normal(s) * 0.05)(B, Sq, D)),
            "k_cache": _w((lambda *s: _rng.normal(s) * 0.05)(B, Hkv, Sk, Dh)),
            "v_cache": _w((lambda *s: _rng.normal(s) * 0.05)(B, Hkv, Sk, Dh)),
            "wq": _w((lambda *s: _rng.normal(s) * 0.05)(D, Hq * Dh) * (D ** -0.5)),
            "wo": _w((lambda *s: _rng.normal(s) * 0.05)(Hq * Dh, D) * ((Hq * Dh) ** -0.5)),
        }
    _A_in = _A_setup()

    def _B_setup():
        B, S, D, F = 1, 1, 640, 1536
        return {
            "x": _w((lambda *s: _rng.normal(s) * 0.05)(B, S, D)),
            "w1": _w((lambda *s: _rng.normal(s) * 0.05)(D, F) * (2.0 / D) ** 0.5),
            "w3": _w((lambda *s: _rng.normal(s) * 0.05)(D, F) * (2.0 / D) ** 0.5),
            "w2": _w((lambda *s: _rng.normal(s) * 0.05)(F, D) * (2.0 / F) ** 0.5),
        }
    _B_in = _B_setup()

    return {
        "A_x": _A_in["x"],
        "A_k_cache": _A_in["k_cache"],
        "A_v_cache": _A_in["v_cache"],
        "A_wq": _A_in["wq"],
        "A_wo": _A_in["wo"],
        "B_x": _B_in["x"],
        "B_w1": _B_in["w1"],
        "B_w3": _B_in["w3"],
        "B_w2": _B_in["w2"],
        "gate_w": _w((lambda *s: _rng.normal(s) * 0.05)(640)),
    }

def reference(A_x, A_k_cache, A_v_cache, A_wq, A_wo, B_x, B_w1, B_w3, B_w2, gate_w):
    def _A_ref(x, k_cache, v_cache, wq, wo):
        B, Sq, D = x.shape
        Hq, Dh = 32, 192
        Hkv, Sk = k_cache.shape[1], k_cache.shape[2]
        W = min(4096, max(256, Sk // 4))
        rep = Hq // Hkv
        q = (lambda x, *d: x.transpose(*d))((x @ wq).reshape(B, Sq, Hq, Dh), 0, 2, 1, 3)
        k = jnp.repeat(k_cache[:, :, Sk - W:, :], rep, axis=1)
        v = jnp.repeat(v_cache[:, :, Sk - W:, :], rep, axis=1)
        scores = jnp.einsum("bhqd,bhkd->bhqk", q, k) * (Dh ** -0.5)
        p = _softmax(scores, axis=-1)
        o = jnp.einsum("bhqk,bhkd->bhqd", p, v)
        return (lambda x, *d: x.transpose(*d))(o, 0, 2, 1, 3).reshape(B, Sq, Hq * Dh) @ wo

    def _B_ref(x, w1, w3, w2):
        gate = jnp.einsum("bsd,df->bsf", x, w1)
        up = jnp.einsum("bsd,df->bsf", x, w3)
        h = _silu(gate) * up
        out = jnp.einsum("bsf,fd->bsd", h, w2)
        return out

    x = A_x
    g = _sigmoid((x * gate_w).sum(-1, keepdims=True))
    a = _A_ref(x, A_k_cache, A_v_cache, A_wq, A_wo)
    b = _B_ref(x, B_w1, B_w3, B_w2)
    return g * a + (1 - g) * b
```

```python
import jax
import jax.numpy as jnp
from jax import lax
import jax.experimental.pallas as pl
import jax.experimental.pallas.tpu as pltpu

_NT = (((1,), (1,)), ((), ()))


@jax.jit
def pallas_gated_mix__sliding_block_cached__glu_gated_swiglu__decode_kernel(
    A_x: jax.Array,
    A_k_cache: jax.Array,
    A_v_cache: jax.Array,
    A_wq: jax.Array,
    A_wo: jax.Array,
    B_x: jax.Array,
    B_w1: jax.Array,
    B_w3: jax.Array,
    B_w2: jax.Array,
    gate_w: jax.Array,
):
    del B_x
    _, H, SK, DH = A_k_cache.shape
    D = A_x.shape[-1]
    F = B_w1.shape[1]
    HD = H * DH
    W = min(4096, max(256, SK // 4))
    S0 = SK - W
    G = 2
    R = G * DH
    NG = H // G
    NB = 3
    PR = R
    NP = HD // PR
    scale = DH ** -0.5

    def kernel(x_hbm, gw_hbm, kT, vT, wq, wo, w1, w3, w2, out_ref,
               kbuf, vbuf, wq_v, wo_v, w1_v, w3_v, w2_v, x_v, gw_v, o_s, b_s, g_s,
               ksem, vsem, wsem, osem):
        def kcopy(g, slot):
            return pltpu.make_async_copy(
                kT.at[pl.ds(pl.multiple_of(g * R, R), R), pl.ds(S0, W)],
                kbuf.at[slot], ksem.at[slot])

        def vcopy(g, slot):
            return pltpu.make_async_copy(
                vT.at[pl.ds(pl.multiple_of(g * R, R), R), pl.ds(S0, W)],
                vbuf.at[slot], vsem.at[slot])

        def wocopy(j):
            r0 = pl.multiple_of(j * PR, PR)
            return pltpu.make_async_copy(
                wo.at[pl.ds(r0, PR), :], wo_v.at[pl.ds(r0, PR), :], osem.at[j])

        x_c = pltpu.make_async_copy(x_hbm, x_v, wsem.at[0])
        gw_c = pltpu.make_async_copy(gw_hbm, gw_v, wsem.at[1])
        w1_c = pltpu.make_async_copy(w1, w1_v, wsem.at[2])
        w3_c = pltpu.make_async_copy(w3, w3_v, wsem.at[3])
        w2_c = pltpu.make_async_copy(w2, w2_v, wsem.at[4])
        wq_c = pltpu.make_async_copy(wq, wq_v, wsem.at[5])

        w1_c.start()
        x_c.start()
        gw_c.start()
        w3_c.start()
        w2_c.start()
        wq_c.start()
        for i in range(NB):
            kcopy(i, i).start()
            vcopy(i, i).start()

        rows = lax.broadcasted_iota(jnp.int32, (8, R), 0)
        cols = lax.broadcasted_iota(jnp.int32, (8, R), 1)
        mask = (cols >= rows * DH) & (cols < (rows + 1) * DH)

        x_c.wait()
        x = x_v[...]
        x8 = jnp.broadcast_to(x, (8, D))
        w1_c.wait()
        gate = jnp.dot(x8, w1_v[...], preferred_element_type=jnp.float32)
        w3_c.wait()
        up = jnp.dot(x8, w3_v[...], preferred_element_type=jnp.float32)
        hid = (gate * jax.nn.sigmoid(gate) * up).astype(jnp.bfloat16)
        w2_c.wait()
        b = jnp.dot(hid, w2_v[...], preferred_element_type=jnp.float32)
        gw_c.wait()
        gw = gw_v[...].astype(jnp.float32).reshape(1, D)
        gl = jnp.sum(x.astype(jnp.float32) * gw, axis=-1, keepdims=True)
        gg = jax.nn.sigmoid(gl)
        b_s[...] = (1.0 - gg) * b
        g_s[...] = jnp.broadcast_to(gg, (8, 128))
        wq_c.wait()

        def step(g, prefetch):
            sl = g % NB
            c0 = pl.multiple_of(g * R, 128)
            qg = jnp.dot(x8, wq_v[:, pl.ds(c0, R)], preferred_element_type=jnp.float32)
            qbd = jnp.where(mask, qg, 0.0).astype(jnp.bfloat16)
            kcopy(g, sl).wait()
            s = jnp.dot(qbd, kbuf[sl], preferred_element_type=jnp.float32) * scale
            if prefetch:
                kcopy(g + NB, sl).start()
            m = jnp.max(s, axis=-1, keepdims=True)
            p = jnp.exp(s - m)
            l = jnp.sum(p, axis=-1, keepdims=True)
            pb = p.astype(jnp.bfloat16)
            vcopy(g, sl).wait()
            o = lax.dot_general(pb, vbuf[sl], _NT, preferred_element_type=jnp.float32)
            if prefetch:
                vcopy(g + NB, sl).start()
            om = jnp.sum(jnp.where(mask, o / l, 0.0), axis=0, keepdims=True)
            o_s[:, pl.ds(c0, R)] = jnp.broadcast_to(om, (8, R))

        def body_pf(g, c):
            step(g, True)
            return c

        def body_np(g, c):
            step(g, False)
            return c

        lax.fori_loop(0, NG - NB, body_pf, 0)

        def wo_start(j, c):
            wocopy(j).start()
            return c

        lax.fori_loop(0, NP, wo_start, 0)
        lax.fori_loop(NG - NB, NG, body_np, 0)

        def obody(j, acc):
            wocopy(j).wait()
            r0 = pl.multiple_of(j * PR, PR)
            return acc + jnp.dot(o_s[:, pl.ds(r0, PR)].astype(jnp.bfloat16),
                                 wo_v[pl.ds(r0, PR), :],
                                 preferred_element_type=jnp.float32)

        acc = lax.fori_loop(0, NP, obody, jnp.zeros((8, D), jnp.float32))
        out_ref[...] = (g_s[0:1, 0:1] * acc[0:1, :] + b_s[0:1, :]).astype(out_ref.dtype)

    hbm = pl.BlockSpec(memory_space=pltpu.HBM)
    kT = jnp.transpose(A_k_cache, (0, 1, 3, 2)).reshape(HD, SK)
    vT = jnp.transpose(A_v_cache, (0, 1, 3, 2)).reshape(HD, SK)
    out = pl.pallas_call(
        kernel,
        out_shape=jax.ShapeDtypeStruct((1, D), A_x.dtype),
        in_specs=[hbm] * 9,
        out_specs=pl.BlockSpec(memory_space=pltpu.VMEM),
        scratch_shapes=[
            pltpu.VMEM((NB, R, W), jnp.bfloat16),
            pltpu.VMEM((NB, R, W), jnp.bfloat16),
            pltpu.VMEM((D, HD), jnp.bfloat16),
            pltpu.VMEM((HD, D), jnp.bfloat16),
            pltpu.VMEM((D, F), jnp.bfloat16),
            pltpu.VMEM((D, F), jnp.bfloat16),
            pltpu.VMEM((F, D), jnp.bfloat16),
            pltpu.VMEM((1, D), jnp.bfloat16),
            pltpu.VMEM((D,), jnp.bfloat16),
            pltpu.VMEM((8, HD), jnp.float32),
            pltpu.VMEM((8, D), jnp.float32),
            pltpu.VMEM((8, 128), jnp.float32),
            pltpu.SemaphoreType.DMA((NB,)),
            pltpu.SemaphoreType.DMA((NB,)),
            pltpu.SemaphoreType.DMA((6,)),
            pltpu.SemaphoreType.DMA((NP,)),
        ],
        compiler_params=pltpu.CompilerParams(vmem_limit_bytes=100 * 1024 * 1024),
    )(A_x.reshape(1, D), gate_w, kT, vT, A_wq, A_wo, B_w1, B_w3, B_w2)
    return out.reshape(1, 1, D)
```

```python
import jax
import jax.numpy as jnp
from jax import lax
import jax.experimental.pallas as pl
import jax.experimental.pallas.tpu as pltpu

_NT = (((1,), (1,)), ((), ()))


@jax.jit
def pallas_gated_mix__sliding_block_cached__glu_gated_swiglu__decode_kernel(
    A_x: jax.Array,
    A_k_cache: jax.Array,
    A_v_cache: jax.Array,
    A_wq: jax.Array,
    A_wo: jax.Array,
    B_x: jax.Array,
    B_w1: jax.Array,
    B_w3: jax.Array,
    B_w2: jax.Array,
    gate_w: jax.Array,
):
    del B_x
    _, H, SK, DH = A_k_cache.shape
    D = A_x.shape[-1]
    F = B_w1.shape[1]
    HD = H * DH
    W = min(4096, max(256, SK // 4))
    S0 = SK - W
    G = 2
    R = G * DH
    NG = H // G
    NB = 3
    MXU_PIECES = (4096, 1024, 512, 256)
    VPU_PIECES = (128, 96, 32)
    BLK = 512
    pieces = MXU_PIECES + VPU_PIECES
    assert sum(pieces) == HD
    NV = sum(VPU_PIECES)
    offs = [sum(pieces[:i]) for i in range(len(pieces))]
    scale = DH**-0.5

    def kernel(x_hbm, gw_hbm, kT, vT, wq, wo, w1, w3, w2, out_ref,
               kbuf, vbuf, wq_v, wo_v, w1_v, w3_v, w2_v, x_v, gw_v,
               o_s, b_s, g_s, oc_s, ksem, vsem, wsem, osem):
        def kcopy(g, slot):
            return pltpu.make_async_copy(
                kT.at[pl.ds(pl.multiple_of(g * R, R), R), pl.ds(S0, W)],
                kbuf.at[slot], ksem.at[slot])

        def vcopy(g, slot):
            return pltpu.make_async_copy(
                vT.at[pl.ds(pl.multiple_of(g * R, R), R), pl.ds(S0, W)],
                vbuf.at[slot], vsem.at[slot])

        def wocopy(j):
            rows_j = pl.ds(offs[j], pieces[j])
            return pltpu.make_async_copy(wo.at[rows_j, :], wo_v.at[rows_j, :], osem.at[j])

        x_c = pltpu.make_async_copy(x_hbm, x_v, wsem.at[0])
        gw_c = pltpu.make_async_copy(gw_hbm, gw_v, wsem.at[1])
        w1_c = pltpu.make_async_copy(w1, w1_v, wsem.at[2])
        w3_c = pltpu.make_async_copy(w3, w3_v, wsem.at[3])
        w2_c = pltpu.make_async_copy(w2, w2_v, wsem.at[4])
        wq_c = pltpu.make_async_copy(wq, wq_v, wsem.at[5])

        w1_c.start()
        x_c.start()
        gw_c.start()
        w3_c.start()
        w2_c.start()
        wq_c.start()
        for i in range(NB):
            kcopy(i, i).start()
            vcopy(i, i).start()

        rows = lax.broadcasted_iota(jnp.int32, (8, R), 0)
        cols = lax.broadcasted_iota(jnp.int32, (8, R), 1)
        mask = (cols >= rows * DH) & (cols < (rows + 1) * DH)

        x_c.wait()
        x = x_v[...]
        x8 = jnp.broadcast_to(x, (8, D))
        w1_c.wait()
        gate = jnp.dot(x8, w1_v[...], preferred_element_type=jnp.float32)
        w3_c.wait()
        up = jnp.dot(x8, w3_v[...], preferred_element_type=jnp.float32)
        hid = (gate * jax.nn.sigmoid(gate) * up).astype(jnp.bfloat16)
        w2_c.wait()
        b = jnp.dot(hid, w2_v[...], preferred_element_type=jnp.float32)
        gw_c.wait()
        gw = gw_v[...].astype(jnp.float32).reshape(1, D)
        gl = jnp.sum(x.astype(jnp.float32) * gw, axis=-1, keepdims=True)
        gg = jax.nn.sigmoid(gl)
        b_s[...] = (1.0 - gg) * b
        g_s[...] = jnp.broadcast_to(gg, (8, D))
        wq_c.wait()

        def head_group(g, carry):
            sl = g % NB

            @pl.when(g == NG - NB)
            def _():
                for j in range(len(pieces)):
                    wocopy(j).start()

            c0 = pl.multiple_of(g * R, 128)
            qg = jnp.dot(x8, wq_v[:, pl.ds(c0, R)], preferred_element_type=jnp.float32)
            qbd = jnp.where(mask, qg, 0.0).astype(jnp.bfloat16)
            kcopy(g, sl).wait()
            s = jnp.dot(qbd, kbuf[sl], preferred_element_type=jnp.float32) * scale

            @pl.when(g + NB < NG)
            def _():
                kcopy(g + NB, sl).start()

            m = jnp.max(s, axis=-1, keepdims=True)
            p = jnp.exp(s - m)
            l = jnp.sum(p, axis=-1, keepdims=True)
            pb = p.astype(jnp.bfloat16)
            vcopy(g, sl).wait()
            o = lax.dot_general(pb, vbuf[sl], _NT, preferred_element_type=jnp.float32)

            @pl.when(g + NB < NG)
            def _():
                vcopy(g + NB, sl).start()

            om = jnp.sum(jnp.where(mask, o / l, 0.0), axis=0, keepdims=True)
            o_s[:, pl.ds(c0, R)] = jnp.broadcast_to(om, (8, R))
            return carry

        lax.fori_loop(0, NG, head_group, 0)

        for t in range(NV // 128):
            c0 = HD - NV + t * 128
            ol = o_s[0:1, c0:c0 + 128].astype(jnp.bfloat16).astype(jnp.float32)
            ol = ol * g_s[0:1, 0:128]
            oc_s[t * 128:(t + 1) * 128, :] = jnp.transpose(jnp.broadcast_to(ol, (128, 128)))

        def out_proj(r0, n, acc):
            return acc + jnp.dot(o_s[:, pl.ds(r0, n)].astype(jnp.bfloat16),
                                 wo_v[pl.ds(r0, n), :],
                                 preferred_element_type=jnp.float32)

        acc = jnp.zeros((8, D), jnp.float32)
        for j in range(len(MXU_PIECES)):
            wocopy(j).wait()
            if pieces[j] > BLK:
                assert pieces[j] % BLK == 0
                acc = lax.fori_loop(
                    0, pieces[j] // BLK,
                    lambda i, a, j=j: out_proj(pl.multiple_of(offs[j] + i * BLK, 128), BLK, a),
                    acc)
            else:
                acc = out_proj(offs[j], pieces[j], acc)

        tot = (g_s[...] * acc + b_s[...]) * 0.125
        for j in range(len(MXU_PIECES), len(pieces)):
            wocopy(j).wait()
            n = pieces[j]
            a = offs[j] - (HD - NV)
            w = wo_v[offs[j]:offs[j] + n, :].astype(jnp.float32)
            oc = jnp.concatenate([oc_s[a:a + n, :]] * (D // 128), axis=1)
            tot = tot + jnp.sum((w * oc).reshape(n // 8, 8, D), axis=0)
        out_ref[...] = jnp.sum(tot, axis=0, keepdims=True).astype(out_ref.dtype)

    hbm = pl.BlockSpec(memory_space=pltpu.HBM)
    kT = jnp.transpose(A_k_cache, (0, 1, 3, 2)).reshape(HD, SK)
    vT = jnp.transpose(A_v_cache, (0, 1, 3, 2)).reshape(HD, SK)
    out = pl.pallas_call(
        kernel,
        out_shape=jax.ShapeDtypeStruct((1, D), A_x.dtype),
        in_specs=[hbm] * 9,
        out_specs=pl.BlockSpec(memory_space=pltpu.VMEM),
        scratch_shapes=[
            pltpu.VMEM((NB, R, W), jnp.bfloat16),
            pltpu.VMEM((NB, R, W), jnp.bfloat16),
            pltpu.VMEM((D, HD), jnp.bfloat16),
            pltpu.VMEM((HD, D), jnp.bfloat16),
            pltpu.VMEM((D, F), jnp.bfloat16),
            pltpu.VMEM((D, F), jnp.bfloat16),
            pltpu.VMEM((F, D), jnp.bfloat16),
            pltpu.VMEM((1, D), jnp.bfloat16),
            pltpu.VMEM((D,), jnp.bfloat16),
            pltpu.VMEM((8, HD), jnp.float32),
            pltpu.VMEM((8, D), jnp.float32),
            pltpu.VMEM((8, D), jnp.float32),
            pltpu.VMEM((NV, 128), jnp.float32),
            pltpu.SemaphoreType.DMA((NB,)),
            pltpu.SemaphoreType.DMA((NB,)),
            pltpu.SemaphoreType.DMA((6,)),
            pltpu.SemaphoreType.DMA((len(pieces),)),
        ],
        compiler_params=pltpu.CompilerParams(
            vmem_limit_bytes=100 * 1024 * 1024,
            disable_semaphore_checks=True,
        ),
    )(A_x.reshape(1, D), gate_w, kT, vT, A_wq, A_wo, B_w1, B_w3, B_w2)
    return out.reshape(1, 1, D)
```

```python
import jax
import jax.numpy as jnp
from jax import lax
import jax.experimental.pallas as pl
import jax.experimental.pallas.tpu as pltpu

_NT = (((1,), (1,)), ((), ()))


@jax.jit
def pallas_gated_mix__sliding_block_cached__glu_gated_swiglu__decode_kernel(
    A_x: jax.Array,
    A_k_cache: jax.Array,
    A_v_cache: jax.Array,
    A_wq: jax.Array,
    A_wo: jax.Array,
    B_x: jax.Array,
    B_w1: jax.Array,
    B_w3: jax.Array,
    B_w2: jax.Array,
    gate_w: jax.Array,
):
    del B_x
    _, H, SK, DH = A_k_cache.shape
    D = A_x.shape[-1]
    F = B_w1.shape[1]
    HD = H * DH
    W = min(4096, max(256, SK // 4))
    S0 = SK - W
    G = 2
    R = G * DH
    NG = H // G
    NB = 2
    NSEM = 2 * NB
    MXU_PIECES = (4096, 1024, 512, 256)
    VPU_PIECES = (128, 96, 32)
    BLK = 512
    pieces = MXU_PIECES + VPU_PIECES
    NP = len(pieces)
    assert sum(pieces) == HD and NP >= NSEM
    NV = sum(VPU_PIECES)
    offs = [sum(pieces[:i]) for i in range(NP)]
    scale = DH**-0.5

    def kernel(x_hbm, gw_hbm, kT, vT, wq, wo, w1, w3, w2, out_ref,
               kbuf, vbuf, wq_v, wo_v, w1_v, w3_v, w2_v, x_v, gw_v,
               o_s, b_s, g_s, oc_s, sem):
        def kcopy(g, slot):
            return pltpu.make_async_copy(
                kT.at[pl.ds(pl.multiple_of(g * R, R), R), pl.ds(S0, W)],
                kbuf.at[slot], sem.at[2 * slot])

        def vcopy(g, slot):
            return pltpu.make_async_copy(
                vT.at[pl.ds(pl.multiple_of(g * R, R), R), pl.ds(S0, W)],
                vbuf.at[slot], sem.at[2 * slot + 1])

        def wocopy(j):
            rows_j = pl.ds(offs[j], pieces[j])
            return pltpu.make_async_copy(wo.at[rows_j, :], wo_v.at[rows_j, :], sem.at[j % NSEM])

        upfront = [
            pltpu.make_async_copy(src, dst, sem.at[2])
            for src, dst in ((w1, w1_v), (x_hbm, x_v), (gw_hbm, gw_v),
                             (w3, w3_v), (w2, w2_v), (wq, wq_v))
        ]
        for c in upfront:
            c.start()
        kcopy(0, 0).start()
        vcopy(0, 0).start()
        vcopy(1, 1).start()

        rows = lax.broadcasted_iota(jnp.int32, (8, R), 0)
        cols = lax.broadcasted_iota(jnp.int32, (8, R), 1)
        mask = (cols >= rows * DH) & (cols < (rows + 1) * DH)

        for c in upfront:
            c.wait()
        kcopy(1, 1).start()

        x = x_v[...]
        x8 = jnp.broadcast_to(x, (8, D))
        gate = jnp.dot(x8, w1_v[...], preferred_element_type=jnp.float32)
        up = jnp.dot(x8, w3_v[...], preferred_element_type=jnp.float32)
        hid = (gate * jax.nn.sigmoid(gate) * up).astype(jnp.bfloat16)
        b = jnp.dot(hid, w2_v[...], preferred_element_type=jnp.float32)
        gw = gw_v[...].astype(jnp.float32).reshape(1, D)
        gl = jnp.sum(x.astype(jnp.float32) * gw, axis=-1, keepdims=True)
        gg = jax.nn.sigmoid(gl)
        b_s[...] = (1.0 - gg) * b
        g_s[...] = jnp.broadcast_to(gg, (8, D))

        def head_group(g, carry):
            sl = g % NB
            c0 = pl.multiple_of(g * R, 128)
            qg = jnp.dot(x8, wq_v[:, pl.ds(c0, R)], preferred_element_type=jnp.float32)
            qbd = jnp.where(mask, qg, 0.0).astype(jnp.bfloat16)
            kcopy(g, sl).wait()
            s = jnp.dot(qbd, kbuf[sl], preferred_element_type=jnp.float32) * scale

            @pl.when(g + NB < NG)
            def _():
                kcopy(g + NB, sl).start()

            for t in range(NB):

                @pl.when(g == NG - NB + t)
                def _():
                    wocopy(2 * t).start()

            m = jnp.max(s, axis=-1, keepdims=True)
            p = jnp.exp(s - m)
            l = jnp.sum(p, axis=-1, keepdims=True)
            pb = p.astype(jnp.bfloat16)
            vcopy(g, sl).wait()
            o = lax.dot_general(pb, vbuf[sl], _NT, preferred_element_type=jnp.float32)

            @pl.when(g + NB < NG)
            def _():
                vcopy(g + NB, sl).start()

            for t in range(NB):

                @pl.when(g == NG - NB + t)
                def _():
                    wocopy(2 * t + 1).start()

            om = jnp.sum(jnp.where(mask, o / l, 0.0), axis=0, keepdims=True)
            o_s[:, pl.ds(c0, R)] = jnp.broadcast_to(om, (8, R))
            return carry

        lax.fori_loop(0, NG, head_group, 0)

        for t in range(NV // 128):
            c0 = HD - NV + t * 128
            ol = o_s[0:1, c0:c0 + 128].astype(jnp.bfloat16).astype(jnp.float32)
            ol = ol * g_s[0:1, 0:128]
            oc_s[t * 128:(t + 1) * 128, :] = jnp.transpose(jnp.broadcast_to(ol, (128, 128)))

        def arrive(j):
            wocopy(j).wait()
            if j + NSEM < NP:
                wocopy(j + NSEM).start()

        def out_proj(r0, n, acc):
            return acc + jnp.dot(o_s[:, pl.ds(r0, n)].astype(jnp.bfloat16),
                                 wo_v[pl.ds(r0, n), :],
                                 preferred_element_type=jnp.float32)

        acc = jnp.zeros((8, D), jnp.float32)
        for j in range(len(MXU_PIECES)):
            arrive(j)
            if pieces[j] > BLK:
                assert pieces[j] % BLK == 0
                acc = lax.fori_loop(
                    0, pieces[j] // BLK,
                    lambda i, a, j=j: out_proj(pl.multiple_of(offs[j] + i * BLK, 128), BLK, a),
                    acc)
            else:
                acc = out_proj(offs[j], pieces[j], acc)

        tot = (g_s[...] * acc + b_s[...]) * 0.125
        for j in range(len(MXU_PIECES), NP):
            arrive(j)
            n = pieces[j]
            a = offs[j] - (HD - NV)
            w = wo_v[offs[j]:offs[j] + n, :].astype(jnp.float32)
            oc = jnp.concatenate([oc_s[a:a + n, :]] * (D // 128), axis=1)
            tot = tot + jnp.sum((w * oc).reshape(n // 8, 8, D), axis=0)
        out_ref[...] = jnp.sum(tot, axis=0, keepdims=True).astype(out_ref.dtype)

    hbm = pl.BlockSpec(memory_space=pltpu.HBM)
    kT = jnp.transpose(A_k_cache, (0, 1, 3, 2)).reshape(HD, SK)
    vT = jnp.transpose(A_v_cache, (0, 1, 3, 2)).reshape(HD, SK)
    out = pl.pallas_call(
        kernel,
        out_shape=jax.ShapeDtypeStruct((1, D), A_x.dtype),
        in_specs=[hbm] * 9,
        out_specs=pl.BlockSpec(memory_space=pltpu.VMEM),
        scratch_shapes=[
            pltpu.VMEM((NB, R, W), jnp.bfloat16),
            pltpu.VMEM((NB, R, W), jnp.bfloat16),
            pltpu.VMEM((D, HD), jnp.bfloat16),
            pltpu.VMEM((HD, D), jnp.bfloat16),
            pltpu.VMEM((D, F), jnp.bfloat16),
            pltpu.VMEM((D, F), jnp.bfloat16),
            pltpu.VMEM((F, D), jnp.bfloat16),
            pltpu.VMEM((1, D), jnp.bfloat16),
            pltpu.VMEM((D,), jnp.bfloat16),
            pltpu.VMEM((8, HD), jnp.float32),
            pltpu.VMEM((8, D), jnp.float32),
            pltpu.VMEM((8, D), jnp.float32),
            pltpu.VMEM((NV, 128), jnp.float32),
            pltpu.SemaphoreType.DMA((NSEM,)),
        ],
        compiler_params=pltpu.CompilerParams(vmem_limit_bytes=64 * 1024 * 1024),
    )(A_x.reshape(1, D), gate_w, kT, vT, A_wq, A_wo, B_w1, B_w3, B_w2)
    return out.reshape(1, 1, D)
```

```python
import functools

import jax
import jax.numpy as jnp
from jax import lax
import jax.experimental.pallas as pl
import jax.experimental.pallas.tpu as pltpu

_NT = (((1,), (1,)), ((), ()))


@jax.jit
def pallas_gated_mix__sliding_block_cached__glu_gated_swiglu__decode_kernel(
    A_x: jax.Array,
    A_k_cache: jax.Array,
    A_v_cache: jax.Array,
    A_wq: jax.Array,
    A_wo: jax.Array,
    B_x: jax.Array,
    B_w1: jax.Array,
    B_w3: jax.Array,
    B_w2: jax.Array,
    gate_w: jax.Array,
):
    del B_x
    _, H, SK, DH = A_k_cache.shape
    D = A_x.shape[-1]
    F = B_w1.shape[1]
    HD = H * DH
    W = min(4096, max(256, SK // 4))
    S0 = SK - W
    G = 2
    R = G * DH
    NG = H // G
    NB = 3
    MXU_PIECES = (4096, 1024, 512, 256)
    VPU_PIECES = (128, 64, 48, 16)
    BLK = 512
    pieces = MXU_PIECES + VPU_PIECES
    NP = len(pieces)
    assert sum(pieces) == HD
    NV = sum(VPU_PIECES)
    offs = [sum(pieces[:i]) for i in range(NP)]
    scale = DH**-0.5

    def main(x_hbm, gw_hbm, kT, vT, wq, wo, w1, w3, w2, out_ref,
             kbuf, vbuf, wq_v, wo_v, w1_v, w3_v, w2_v, x_v, gw_v,
             o_s, b_s, g_s, oc_s, ksem, vsem, wsem, osem):
        def kcopy(g, slot):
            return pltpu.make_async_copy(
                kT.at[pl.ds(pl.multiple_of(g * R, R), R), pl.ds(S0, W)],
                kbuf.at[slot], ksem.at[slot])

        def vcopy(g, slot):
            return pltpu.make_async_copy(
                vT.at[pl.ds(pl.multiple_of(g * R, R), R), pl.ds(S0, W)],
                vbuf.at[slot], vsem.at[slot])

        def wocopy(j):
            rows_j = pl.ds(offs[j], pieces[j])
            return pltpu.make_async_copy(wo.at[rows_j, :], wo_v.at[rows_j, :], osem.at[j])

        x_c = pltpu.make_async_copy(x_hbm, x_v, wsem.at[0])
        gw_c = pltpu.make_async_copy(gw_hbm, gw_v, wsem.at[1])
        w1_c = pltpu.make_async_copy(w1, w1_v, wsem.at[2])
        w3_c = pltpu.make_async_copy(w3, w3_v, wsem.at[3])
        w2_c = pltpu.make_async_copy(w2, w2_v, wsem.at[4])
        wq_c = pltpu.make_async_copy(wq, wq_v, wsem.at[5])

        w1_c.start()
        x_c.start()
        gw_c.start()
        w3_c.start()
        w2_c.start()
        wq_c.start()
        for i in range(NB):
            kcopy(i, i).start()
            vcopy(i, i).start()

        rows = lax.broadcasted_iota(jnp.int32, (8, R), 0)
        cols = lax.broadcasted_iota(jnp.int32, (8, R), 1)
        mask = (cols >= rows * DH) & (cols < (rows + 1) * DH)

        x_c.wait()
        x = x_v[...]
        x8 = jnp.broadcast_to(x, (8, D))
        w1_c.wait()
        gate = jnp.dot(x8, w1_v[...], preferred_element_type=jnp.float32)
        w3_c.wait()
        up = jnp.dot(x8, w3_v[...], preferred_element_type=jnp.float32)
        hid = (gate * jax.nn.sigmoid(gate) * up).astype(jnp.bfloat16)
        w2_c.wait()
        b = jnp.dot(hid, w2_v[...], preferred_element_type=jnp.float32)
        gw_c.wait()
        gw = gw_v[...].astype(jnp.float32).reshape(1, D)
        gl = jnp.sum(x.astype(jnp.float32) * gw, axis=-1, keepdims=True)
        gg = jax.nn.sigmoid(gl)
        b_s[...] = (1.0 - gg) * b
        g_s[...] = jnp.broadcast_to(gg, (8, D))
        wq_c.wait()

        def head_group(g, carry):
            sl = g % NB

            @pl.when(g == NG - NB)
            def _():
                for j in range(NP):
                    wocopy(j).start()

            c0 = pl.multiple_of(g * R, 128)
            qg = jnp.dot(x8, wq_v[:, pl.ds(c0, R)], preferred_element_type=jnp.float32)
            qbd = jnp.where(mask, qg, 0.0).astype(jnp.bfloat16)
            kcopy(g, sl).wait()
            s = jnp.dot(qbd, kbuf[sl], preferred_element_type=jnp.float32) * scale

            @pl.when(g + NB < NG)
            def _():
                kcopy(g + NB, sl).start()

            m = jnp.max(s, axis=-1, keepdims=True)
            p = jnp.exp(s - m)
            l = jnp.sum(p, axis=-1, keepdims=True)
            pb = p.astype(jnp.bfloat16)
            vcopy(g, sl).wait()
            o = lax.dot_general(pb, vbuf[sl], _NT, preferred_element_type=jnp.float32)

            @pl.when(g + NB < NG)
            def _():
                vcopy(g + NB, sl).start()

            om = jnp.sum(jnp.where(mask, o / l, 0.0), axis=0, keepdims=True)
            o_s[:, pl.ds(c0, R)] = jnp.broadcast_to(om, (8, R))
            return carry

        lax.fori_loop(0, NG, head_group, 0)

        for t in range(NV // 128):
            c0 = HD - NV + t * 128
            ol = o_s[0:1, c0:c0 + 128].astype(jnp.bfloat16).astype(jnp.float32)
            ol = ol * g_s[0:1, 0:128]
            oc_s[t * 128:(t + 1) * 128, :] = jnp.transpose(jnp.broadcast_to(ol, (128, 128)))

        def out_proj(r0, n, acc):
            return acc + jnp.dot(o_s[:, pl.ds(r0, n)].astype(jnp.bfloat16),
                                 wo_v[pl.ds(r0, n), :],
                                 preferred_element_type=jnp.float32)

        acc = jnp.zeros((8, D), jnp.float32)
        for j in range(len(MXU_PIECES)):
            wocopy(j).wait()
            if pieces[j] > BLK:
                assert pieces[j] % BLK == 0
                acc = lax.fori_loop(
                    0, pieces[j] // BLK,
                    lambda i, a, j=j: out_proj(pl.multiple_of(offs[j] + i * BLK, 128), BLK, a),
                    acc)
            else:
                acc = out_proj(offs[j], pieces[j], acc)

        tot = (g_s[...] * acc + b_s[...]) * 0.125
        for j in range(len(MXU_PIECES), NP):
            wocopy(j).wait()
            n = pieces[j]
            a = offs[j] - (HD - NV)
            w = wo_v[offs[j]:offs[j] + n, :].astype(jnp.float32)
            oc = jnp.concatenate([oc_s[a:a + n, :]] * (D // 128), axis=1)
            tot = tot + jnp.sum((w * oc).reshape(n // 8, 8, D), axis=0)
        out_ref[...] = jnp.sum(tot, axis=0, keepdims=True).astype(out_ref.dtype)

    def kernel(*refs):
        pl.run_scoped(
            functools.partial(main, *refs),
            pltpu.SemaphoreType.DMA((NB,)),
            pltpu.SemaphoreType.DMA((NB,)),
            pltpu.SemaphoreType.DMA((6,)),
            pltpu.SemaphoreType.DMA((NP,)),
        )

    hbm = pl.BlockSpec(memory_space=pltpu.HBM)
    kT = jnp.transpose(A_k_cache, (0, 1, 3, 2)).reshape(HD, SK)
    vT = jnp.transpose(A_v_cache, (0, 1, 3, 2)).reshape(HD, SK)
    out = pl.pallas_call(
        kernel,
        out_shape=jax.ShapeDtypeStruct((1, D), A_x.dtype),
        in_specs=[hbm] * 9,
        out_specs=pl.BlockSpec(memory_space=pltpu.VMEM),
        scratch_shapes=[
            pltpu.VMEM((NB, R, W), jnp.bfloat16),
            pltpu.VMEM((NB, R, W), jnp.bfloat16),
            pltpu.VMEM((D, HD), jnp.bfloat16),
            pltpu.VMEM((HD, D), jnp.bfloat16),
            pltpu.VMEM((D, F), jnp.bfloat16),
            pltpu.VMEM((D, F), jnp.bfloat16),
            pltpu.VMEM((F, D), jnp.bfloat16),
            pltpu.VMEM((1, D), jnp.bfloat16),
            pltpu.VMEM((D,), jnp.bfloat16),
            pltpu.VMEM((8, HD), jnp.float32),
            pltpu.VMEM((8, D), jnp.float32),
            pltpu.VMEM((8, D), jnp.float32),
            pltpu.VMEM((NV, 128), jnp.float32),
        ],
        compiler_params=pltpu.CompilerParams(vmem_limit_bytes=64 * 1024 * 1024),
    )(A_x.reshape(1, D), gate_w, kT, vT, A_wq, A_wo, B_w1, B_w3, B_w2)
    return out.reshape(1, 1, D)
```
